```python
import jax
import jax.numpy as jnp

def _softmax(x, axis=-1):
    return jax.nn.softmax(x, axis=axis)
def _gelu(x):
    return jax.nn.gelu(x, approximate=True)
def _silu(x):
    return jax.nn.silu(x)
def _sigmoid(x):
    return jax.nn.sigmoid(x)
def _layernorm(x, axis=-1, eps=1e-5):
    m = jnp.mean(x, axis=axis, keepdims=True)
    v = jnp.var(x, axis=axis, keepdims=True)
    return (x - m) / jnp.sqrt(v + eps)
def _scatter_add(tgt, idx, src, axis=0):
    return tgt.at[idx].add(src)
def _segment_sum(src, seg, n):
    return jax.ops.segment_sum(src, seg, n)
class _Rng:
    def __init__(self, key):
        self._k = key
    def _next(self):
        self._k, sub = jax.random.split(self._k)
        return sub
    def normal(self, shape):
        return jax.random.normal(self._next(), shape, dtype=jnp.bfloat16)
    def randint(self, lo, hi, shape):
        return jax.random.randint(self._next(), shape, lo, hi, dtype=jnp.int32)
    def uniform(self, shape, lo=0.0, hi=1.0):
        return jax.random.uniform(self._next(), shape, jnp.bfloat16, lo, hi)
    def permutation(self, n):
        return jax.random.permutation(self._next(), n)


kernel_name = 'gated_mix__compressed_kv_cla__ssm_conv_h3__prompt'

def setup_inputs():
    _rng = _Rng(jax.random.key(int.from_bytes(__import__("os").urandom(4), "little")))
    _w = (lambda a: (lambda t: t.astype(jnp.bfloat16) if jnp.issubdtype(t.dtype, jnp.floating) else t)(jnp.asarray(a)))
    def _A_setup():
        B, H, Sq, Sk, D, M = 1, 32, 2048, 2048, 128, 1024
        Dc = 4 * D
        return {
            "x": _w((lambda *s: _rng.normal(s) * 0.05)(B, Sq, M)),
            "c_kv": _w((lambda *s: _rng.normal(s) * 0.05)(B, Sk, Dc)),
            "w_q": _w((lambda *s: _rng.normal(s) * 0.05)(M, H, D) * (M ** -0.5)),
            "w_uk": _w((lambda *s: _rng.normal(s) * 0.05)(Dc, H, D) * (Dc ** -0.5)),
            "w_uv": _w((lambda *s: _rng.normal(s) * 0.05)(Dc, H, D) * (Dc ** -0.5)),
            "w_o": _w((lambda *s: _rng.normal(s) * 0.05)(H, D, M) * ((H * D) ** -0.5)),
        }
    _A_in = _A_setup()

    def _B_setup():
        B, S, D = 1, 2048, 1024
        ks = 4
        return {
            "q": _w((lambda *s: _rng.normal(s) * 0.05)(B, S, D)),
            "k": _w((lambda *s: _rng.normal(s) * 0.05)(B, S, D)),
            "v": _w((lambda *s: _rng.normal(s) * 0.05)(B, S, D)),
            "shift_k": _w((lambda *s: _rng.normal(s) * 0.05)(D, ks) * 0.5),
            "ssm_k": _w((lambda *s: _rng.normal(s) * 0.05)(D, S) * (1.0 / S ** 0.5)),
            "ssm_D": _w((lambda *s: _rng.normal(s) * 0.05)(D)),
        }
    _B_in = _B_setup()

    return {
        "A_x": _A_in["x"],
        "A_c_kv": _A_in["c_kv"],
        "A_w_q": _A_in["w_q"],
        "A_w_uk": _A_in["w_uk"],
        "A_w_uv": _A_in["w_uv"],
        "A_w_o": _A_in["w_o"],
        "B_q": _B_in["q"],
        "B_k": _B_in["k"],
        "B_v": _B_in["v"],
        "B_shift_k": _B_in["shift_k"],
        "B_ssm_k": _B_in["ssm_k"],
        "B_ssm_D": _B_in["ssm_D"],
        "gate_w": _w((lambda *s: _rng.normal(s) * 0.05)(1024)),
    }

def reference(A_x, A_c_kv, A_w_q, A_w_uk, A_w_uv, A_w_o, B_q, B_k, B_v, B_shift_k, B_ssm_k, B_ssm_D, gate_w):
    def _A_ref(x, c_kv, w_q, w_uk, w_uv, w_o):
        B, Sq, M = x.shape[0], x.shape[1], x.shape[2]
        Sk = c_kv.shape[1]
        H, D = w_q.shape[1], w_q.shape[2]
        q = jnp.einsum("bqm,mhd->bhqd", x, w_q)
        k = jnp.einsum("bkc,chd->bhkd", c_kv, w_uk)
        v = jnp.einsum("bkc,chd->bhkd", c_kv, w_uv)
        scores = jnp.einsum("bhqd,bhkd->bhqk", q, k) * (D ** -0.5)
        off = Sk - Sq
        qi = jnp.arange(Sq)[:, None]
        kj = jnp.arange(Sk)[None, :]
        cmask = kj <= (qi + off)
        scores = jnp.where(cmask[None, None], scores, -1e9)
        p = _softmax(scores, axis=-1)
        ctx = jnp.einsum("bhqk,bhkd->bhqd", p, v)
        return jnp.einsum("bhqd,hdm->bqm", ctx, w_o)

    def _B_ref(q, k, v, shift_k, ssm_k, ssm_D):
        B, S, D = q.shape
        ks = shift_k.shape[-1]
        k_pad = jnp.pad(k, ((0, 0), (ks - 1, 0), (0, 0)))
        k_shift = jnp.zeros_like(k)
        for t in range(ks):
            k_shift = k_shift + k_pad[:, t:t + S, :] * shift_k[:, ks - 1 - t][None, None, :]
        kv = k_shift * v
        L = 2 * S
        kv_pad = jnp.pad(kv, ((0, 0), (0, S), (0, 0)))
        kf_pad = jnp.pad(ssm_k, ((0, 0), (0, S)))
        kv_f = (lambda x, axes=(-2,-1): jnp.fft.rfft2(x.astype(jnp.float32), axes=axes))(kv_pad[:, None, :, :], axes=(1, 2))
        kf_f = (lambda x, axes=(-2,-1): jnp.fft.rfft2(x.astype(jnp.float32), axes=axes))(kf_pad[:, None, :], axes=(1, 2))
        kf_f = (lambda x, *d: x.transpose(*d))(kf_f, 1, 2, 0)
        y_f = kv_f * kf_f[None, :, :, :]
        y = (lambda x, s, axes=(-2,-1): jnp.fft.irfft2(x, s=s, axes=axes).astype(jnp.bfloat16))(y_f, (1, L), axes=(1, 2))[:, 0, :S, :]
        y = y + kv * ssm_D[None, None, :]
        return q * y

    x = A_x
    g = _sigmoid((x * gate_w).sum(-1, keepdims=True))
    a = _A_ref(x, A_c_kv, A_w_q, A_w_uk, A_w_uv, A_w_o)
    b = _B_ref(x, B_k, B_v, B_shift_k, B_ssm_k, B_ssm_D)
    return g * a + (1 - g) * b
```

```python
import numpy as np
import jax
import jax.numpy as jnp
import jax.experimental.pallas as pl
import jax.experimental.pallas.tpu as pltpu

S, M, H, D, DC = 2048, 1024, 32, 128, 512
P = 128
NP = S // P
NG = M // 128
BQ = 256
F32, BF16 = jnp.float32, jnp.bfloat16
NT = (((1,), (1,)), ((), ()))


def _dft():
    w = 2 * np.pi * (np.arange(P)[:, None] + 0.5) * np.arange(P)[None, :] / (2 * P)
    f = np.concatenate([np.cos(w), -np.sin(w)], 0)
    return f.astype(np.float32), np.ascontiguousarray(f.T / P).astype(np.float32)


def _dot(a, b):
    return jnp.dot(a, b, preferred_element_type=F32)


def _kernel(x_ref, c_ref, wq_ref, wk_ref, wv_ref, wo_ref, xb_ref, k_ref, v_ref,
            sk_ref, ssm_ref, sd_ref, gw_ref, f_ref, fi_ref, o_ref,
            acc, q_s, k_s, v_s, s_s, g_s, kp_s, xf_s, hf_s, w_s):
    step = pl.program_id(0)

    @pl.when(step == 0)
    def _init():
        acc[...] = jnp.zeros(acc.shape, F32)

    def split(h):
        sh = (16 * (1 - h % 2)).astype(jnp.uint32)
        for ref, o in ((wq_ref, 0), (wk_ref, M), (wv_ref, M + DC)):
            u = ref.bitcast(jnp.uint32)[:, (h % 16) // 2, :]
            u = (u << sh) & jnp.uint32(0xFFFF0000)
            w_s[h % 2, o:o + u.shape[0], :] = pltpu.bitcast(u, F32).astype(BF16)

    pl.when(step == 0)(lambda: split(step))

    @pl.when(step < H)
    def _attn():
        wq, wk, wv = w_s[step % 2, :M], w_s[step % 2, M:M + DC], w_s[step % 2, M + DC:]
        scale = D ** -0.5 * np.log2(np.e)
        for r in range(0, S, 512):
            rows = slice(r, r + 512)
            q_s[rows, :] = (_dot(x_ref[rows, :], wq) * scale).astype(BF16)
            k_s[rows, :] = _dot(c_ref[rows, :], wk).astype(BF16)
            v_s[rows, :] = _dot(c_ref[rows, :], wv).astype(BF16)
        split(jnp.minimum(step + 1, H - 1))
        ri = jax.lax.broadcasted_iota(jnp.int32, (128, 128), 0)
        ci = jax.lax.broadcasted_iota(jnp.int32, (128, 128), 1)
        tri = ci <= ri
        for i in range(S // BQ):
            r0 = i * BQ
            q = q_s[r0:r0 + BQ, :]
            nt = (r0 + BQ) // 128
            m = None
            for j in range(nt):
                d = j * 128 - r0
                if d < 0:
                    s = jax.lax.dot_general(q, k_s[j * 128:j * 128 + 128, :], NT, preferred_element_type=F32)
                elif d == 0:
                    s = jax.lax.dot_general(q, k_s[j * 128:j * 128 + 128, :], NT, preferred_element_type=F32)
                    s = jnp.concatenate([jnp.where(tri, s[:128], -1e30), s[128:]], 0)
                else:
                    s = jax.lax.dot_general(q[128:], k_s[j * 128:j * 128 + 128, :], NT, preferred_element_type=F32)
                    s = jnp.where(tri, s, -1e30)
                if d > 0:
                    s_s[j, 128:, :] = s
                    m = jnp.concatenate([m[:128], jnp.maximum(m[128:], s)], 0)
                else:
                    s_s[j] = s
                    m = s if m is None else jnp.maximum(m, s)
            m = jnp.broadcast_to(jnp.max(m, axis=1, keepdims=True), (BQ, 128))
            o = None
            l = None
            for j in range(nt):
                d = j * 128 - r0
                vt = v_s[j * 128:j * 128 + 128, :]
                if d > 0:
                    p = jnp.exp2(s_s[j, 128:, :] - m[128:])
                    l = jnp.concatenate([l[:128], l[128:] + p], 0)
                    o = jnp.concatenate([o[:128], o[128:] + _dot(p.astype(BF16), vt)], 0)
                else:
                    p = jnp.exp2(s_s[j] - m)
                    l = p if l is None else l + p
                    t = _dot(p.astype(BF16), vt)
                    o = t if o is None else o + t
            ctx = (o / jnp.sum(l, axis=1, keepdims=True)).astype(BF16)
            y = _dot(ctx, wo_ref[...])
            for g in range(NG):
                acc[g, r0:r0 + BQ, :] += y[:, g * 128:(g + 1) * 128]

    @pl.when(step == H)
    def _gate():
        for r in range(0, S, 256):
            t = (x_ref[r:r + 256, :] * gw_ref[...]).astype(F32)
            g = jax.nn.sigmoid(jnp.sum(t, axis=1, keepdims=True))
            g_s[r:r + 256, :] = jnp.broadcast_to(g, (256, 128))

    @pl.when(step >= H)
    def _ssm():
        kp_s[0:8, :] = jnp.zeros((8, 128), F32)
        kp_s[8:, :] = k_ref[...].astype(F32)
        sk = sk_ref[...].astype(F32)
        f = f_ref[...]
        sgn = (1 - 2 * (jax.lax.broadcasted_iota(jnp.int32, (P, 128), 0) & 1)).astype(F32)
        for a in range(NP):
            ks = None
            for t in range(4):
                u = kp_s[8 + a * P - t:8 + (a + 1) * P - t, :] * sk[t:t + 1, :]
                ks = u if ks is None else ks + u
            kv = ks * v_ref[a * P:(a + 1) * P, :].astype(F32)
            xf_s[a] = _dot(f, kv.astype(BF16))
            hf_s[NP + a, 0:P, :] = kv
        prev = None
        for a in range(NP):
            kf = jax.lax.dot_general(f, ssm_ref[:, a * P:(a + 1) * P], NT, preferred_element_type=F32)
            if prev is None:
                hf_s[a] = kf
            else:
                hf_s[a, 0:P, :] = kf[:P] - sgn * prev[P:]
                hf_s[a, P:, :] = kf[P:] + sgn * prev[:P]
            prev = kf
        sd = sd_ref[...].astype(F32)
        for j in range(NP):
            zs = []
            for r in range(0, P, 32):
                zr = zi = None
                for i in range(j + 1):
                    xr, xi = xf_s[i, r:r + 32, :], xf_s[i, P + r:P + r + 32, :]
                    hr, hi = hf_s[j - i, r:r + 32, :], hf_s[j - i, P + r:P + r + 32, :]
                    tr, ti = xr * hr - xi * hi, xr * hi + xi * hr
                    zr, zi = (tr, ti) if zr is None else (zr + tr, zi + ti)
                zs.append((zr, zi))
            z = jnp.concatenate([t[0] for t in zs] + [t[1] for t in zs], 0).astype(BF16)
            rows = slice(j * P, (j + 1) * P)
            y = _dot(fi_ref[...], z) + hf_s[NP + j, 0:P, :] * sd
            b = xb_ref[rows, :].astype(F32) * y
            g = g_s[rows, :]
            o_ref[rows, :] = (g * acc[step - H, rows, :] + (1 - g) * b).astype(BF16)


@jax.jit
def pallas_gated_mix__compressed_kv_cla__ssm_conv_h3__prompt_kernel(
        A_x, A_c_kv, A_w_q, A_w_uk, A_w_uv, A_w_o, B_q, B_k, B_v, B_shift_k, B_ssm_k, B_ssm_D, gate_w):
    f, fi = _dft()
    hd = lambda s: jnp.minimum(s, H - 1)
    gr = lambda s: jnp.maximum(s - H, 0)
    full = lambda shp: pl.BlockSpec(shp, lambda s: (0,) * len(shp))
    col = pl.BlockSpec((S, 128), lambda s: (0, gr(s)))
    x = A_x.reshape(S, M)
    out = pl.pallas_call(
        _kernel,
        grid=(H + NG,),
        in_specs=[
            full((S, M)), full((S, DC)),
            pl.BlockSpec((M, 16, D), lambda s: (0, hd(s + 1) // 16, 0)),
            pl.BlockSpec((DC, 16, D), lambda s: (0, hd(s + 1) // 16, 0)),
            pl.BlockSpec((DC, 16, D), lambda s: (0, hd(s + 1) // 16, 0)),
            pl.BlockSpec((None, D, M), lambda s: (hd(s), 0, 0)),
            col, col, col,
            pl.BlockSpec((4, 128), lambda s: (0, gr(s))),
            pl.BlockSpec((128, S), lambda s: (gr(s), 0)),
            pl.BlockSpec((1, 128), lambda s: (0, gr(s))),
            full((1, M)), full((2 * P, P)), full((P, 2 * P)),
        ],
        out_specs=col,
        out_shape=jax.ShapeDtypeStruct((S, M), BF16),
        scratch_shapes=[
            pltpu.VMEM((NG, S, 128), F32),
            pltpu.VMEM((S, D), BF16), pltpu.VMEM((S, D), BF16), pltpu.VMEM((S, D), BF16),
            pltpu.VMEM((S // 128, BQ, 128), F32),
            pltpu.VMEM((S, 128), F32),
            pltpu.VMEM((S + 8, 128), F32),
            pltpu.VMEM((NP, 2 * P, 128), F32),
            pltpu.VMEM((2 * NP, 2 * P, 128), F32),
            pltpu.VMEM((2, M + 2 * DC, D), BF16),
        ],
        compiler_params=pltpu.CompilerParams(
            dimension_semantics=("arbitrary",), vmem_limit_bytes=100 * 2**20),
    )(x, A_c_kv.reshape(S, DC), A_w_q, A_w_uk,
      A_w_uv, A_w_o, x, B_k.reshape(S, M), B_v.reshape(S, M),
      B_shift_k.T, B_ssm_k, B_ssm_D.reshape(1, M), gate_w.reshape(1, M), f.astype(BF16), fi.astype(BF16))
    return out.reshape(1, S, M)
```
